```python
import os as _os
_os.environ.setdefault('JAX_PLATFORMS', 'cpu')
import jax
import jax.numpy as jnp

def _softmax(x, axis=-1):
    return jax.nn.softmax(x, axis=axis)

def _gelu(x):
    return jax.nn.gelu(x, approximate=True)

def _silu(x):
    return jax.nn.silu(x)

def _sigmoid(x):
    return jax.nn.sigmoid(x)

def _layernorm(x, axis=-1, eps=1e-05):
    m = jnp.mean(x, axis=axis, keepdims=True)
    v = jnp.var(x, axis=axis, keepdims=True)
    return (x - m) / jnp.sqrt(v + eps)

def _scatter_add(tgt, idx, src, axis=0):
    return tgt.at[idx].add(src)

def _segment_sum(src, seg, n):
    return jax.ops.segment_sum(src, seg, n)

class _Rng:

    def __init__(self, key):
        self._k = key

    def _next(self):
        self._k, sub = jax.random.split(self._k)
        return sub

    def normal(self, shape):
        return jax.random.normal(self._next(), shape, dtype=jnp.bfloat16)

    def randint(self, lo, hi, shape):
        return jax.random.randint(self._next(), shape, lo, hi, dtype=jnp.int32)

    def uniform(self, shape, lo=0.0, hi=1.0):
        return jax.random.uniform(self._next(), shape, jnp.bfloat16, lo, hi)

    def permutation(self, n):
        return jax.random.permutation(self._next(), n)
kernel_name = 'adaLN_cond__linear_kernel_hedgehog__geglu_ffn__prompt'

def setup_inputs():
    _rng = _Rng(jax.random.key(int.from_bytes(__import__("os").urandom(4), "little")))
    _w = lambda a: (lambda t: t.astype(jnp.bfloat16) if jnp.issubdtype(t.dtype, jnp.floating) else t)(jnp.asarray(a))

    def _A_setup():
        B, S, D, H = (1, 2048, 512, 32)
        Dh = D // H
        return {'x': _w((lambda *s: _rng.normal(s) * 0.05)(B, S, D)), 'wqkv': _w((lambda *s: _rng.normal(s) * 0.4)(D, 3 * D)), 'w_phi': _w((lambda *s: _rng.normal(s) * 0.4)(H, Dh, Dh) * Dh ** (-0.5)), 'wo': _w((lambda *s: _rng.normal(s) * 0.05)(D, D))}
    _A_in = _A_setup()

    def _B_setup():
        B, S, D, F = (1, 2048, 512, 1792)
        return {'x': _w((lambda *s: _rng.normal(s) * 0.05)(B, S, D)), 'w_gate': _w((lambda *s: _rng.normal(s) * 0.05)(D, F)), 'w_up': _w((lambda *s: _rng.normal(s) * 0.05)(D, F)), 'w_down': _w((lambda *s: _rng.normal(s) * 0.05)(F, D))}
    _B_in = _B_setup()
    return {'A_x': _A_in['x'], 'A_wqkv': _A_in['wqkv'], 'A_w_phi': _A_in['w_phi'], 'A_wo': _A_in['wo'], 'B_x': _B_in['x'], 'B_w_gate': _B_in['w_gate'], 'B_w_up': _B_in['w_up'], 'B_w_down': _B_in['w_down'], 'c': _w((lambda *s: _rng.normal(s) * 0.05)(1, 512) * 8.0), 'w_mod': _w((lambda *s: _rng.normal(s) * 0.05)(512, 6 * 512) * 512 ** (-0.5) * 8.0)}

def reference(A_x, A_wqkv, A_w_phi, A_wo, B_x, B_w_gate, B_w_up, B_w_down, c, w_mod):

    def _A_ref(x, wqkv, w_phi, wo):
        B, S, D = x.shape
        H = 32
        Dh = D // H
        qkv = (lambda x, *d: x.transpose(*d))((x @ wqkv).reshape(B, S, 3, H, Dh), 2, 0, 3, 1, 4)
        q, k, v = (qkv[0], qkv[1], qkv[2])
        pq = jnp.einsum('bhsd,hdf->bhsf', q, w_phi)
        pk = jnp.einsum('bhsd,hdf->bhsf', k, w_phi)
        phi_q = jnp.concatenate([_softmax(pq, axis=-1), _softmax(-pq, axis=-1)], axis=-1)
        phi_k = jnp.concatenate([_softmax(pk, axis=-1), _softmax(-pk, axis=-1)], axis=-1)
        kv = jnp.einsum('bhsf,bhsd->bhfd', phi_k, v)
        z = jnp.einsum('bhsf->bhf', phi_k)
        num = jnp.einsum('bhqf,bhfd->bhqd', phi_q, kv)
        den = jnp.einsum('bhqf,bhf->bhq', phi_q, z)[..., None] + 1e-06
        o = num / den
        return (lambda x, *d: x.transpose(*d))(o, 0, 2, 1, 3).reshape(B, S, D) @ wo

    def _B_ref(x, w_gate, w_up, w_down):
        return _gelu(x @ w_gate) * (x @ w_up) @ w_down
    x = A_x
    mod = (_silu(c) @ w_mod).reshape(c.shape[0], 6, 1, -1)
    sa, ca, ga, sb, cb, gb = (mod[:, 0].copy(), mod[:, 1].copy(), mod[:, 2].copy(), mod[:, 3].copy(), mod[:, 4].copy(), mod[:, 5].copy())
    h = _layernorm(x, axis=-1) * (1 + ca) + sa
    x = x + ga * _A_ref(h, A_wqkv, A_w_phi, A_wo)
    h = _layernorm(x, axis=-1) * (1 + cb) + sb
    x = x + gb * _B_ref(h, B_w_gate, B_w_up, B_w_down)
    return x
```

```python
import functools

import jax
import jax.numpy as jnp
import jax.experimental.pallas as pl
import jax.experimental.pallas.tpu as pltpu

F32 = jnp.float32
BF16 = jnp.bfloat16

LOG2E = 1.4426950408889634

_NT = (((1,), (1,)), ((), ()))
_TN = (((0,), (0,)), ((), ()))


def _dot(a, b):
    return jnp.dot(a, b, preferred_element_type=F32)


def _dot_nt(a, b):
    return jax.lax.dot_general(a, b, _NT, preferred_element_type=F32)


def _dot_tn(a, b):
    return jax.lax.dot_general(a, b, _TN, preferred_element_type=F32)


def _iota(shape, dim):
    return jax.lax.broadcasted_iota(jnp.int32, shape, dim)


def _layernorm(x, eps=1e-5):
    m = jnp.mean(x, axis=-1, keepdims=True)
    xc = x - m
    v = jnp.mean(xc * xc, axis=-1, keepdims=True)
    return xc * jax.lax.rsqrt(v + eps)


def _gelu_tanh(x):
    c0 = 0.7978845608028654
    return 0.5 * x * (1.0 + jnp.tanh(c0 * (x + 0.044715 * (x * x * x))))


def _make_kernel(S, D, H, Dh, F, TM1, TM2, FC, RC, SCHED, UNR2):
    G = D // 128
    HQ = 4
    QW = HQ * Dh
    NQ = H // HQ
    n1 = S // TM1
    n2 = S // TM2
    NF = F // FC
    NL = TM1 // 128
    NC = TM2 // RC
    LR = QW + 16

    SEM_C, SEM_WPHI, SEM_WQ, SEM_WK, SEM_MODA, SEM_WV = 0, 1, 2, 3, 4, 5
    SEM_MODB, SEM_WO, SEM_WG, SEM_WU, SEM_WD = 6, 7, 8, 9, 10
    SEM_X = 11
    SEM_OUT = SEM_X + n1
    NSEM = SEM_OUT + n2

    def kernel(x_hbm, wqkv_hbm, wphi_hbm, wo_hbm, wg_hbm, wu_hbm, wd_hbm, c_hbm, wmod_hbm,
               out_hbm,
               x_buf, wqkv_buf, wphi_buf, wo_buf, wg_buf, wu_buf, wd_buf, c_buf, wmod_buf,
               w3t_buf, phq_buf, kv_acc, z_acc, lhs_buf, wop_buf, mod_buf,
               h_buf, x1_buf, acc_buf, out_buf, sems):

        def cp(src, dst, slot):
            return pltpu.make_async_copy(src, dst, sems.at[slot])

        c_cp = cp(c_hbm, c_buf, SEM_C)
        wphi_cp = cp(wphi_hbm, wphi_buf, SEM_WPHI)
        wq_cp = cp(wqkv_hbm.at[:, pl.ds(0, D)], wqkv_buf.at[:, pl.ds(0, D)], SEM_WQ)
        wk_cp = cp(wqkv_hbm.at[:, pl.ds(D, D)], wqkv_buf.at[:, pl.ds(D, D)], SEM_WK)
        wv_cp = cp(wqkv_hbm.at[:, pl.ds(2 * D, D)], wqkv_buf.at[:, pl.ds(2 * D, D)], SEM_WV)
        moda_cp = cp(wmod_hbm.at[:, pl.ds(0, 2 * D)], wmod_buf.at[:, pl.ds(0, 2 * D)], SEM_MODA)
        modb_cp = cp(wmod_hbm.at[:, pl.ds(2 * D, 4 * D)], wmod_buf.at[:, pl.ds(2 * D, 4 * D)],
                     SEM_MODB)
        wo_cp = cp(wo_hbm, wo_buf, SEM_WO)
        wg_cp = cp(wg_hbm, wg_buf, SEM_WG)
        wu_cp = cp(wu_hbm, wu_buf, SEM_WU)
        wd_cp = cp(wd_hbm, wd_buf, SEM_WD)

        def x_cp(i):
            r = pl.multiple_of(i * TM1, TM1)
            return cp(x_hbm.at[pl.ds(r, TM1), :], x_buf.at[pl.ds(r, TM1), :], SEM_X + i)

        def out_cp(i):
            r = pl.multiple_of(i * TM2, TM2)
            return cp(out_buf.at[pl.ds(r, TM2), :], out_hbm.at[pl.ds(r, TM2), :], SEM_OUT + i)

        wphi_cp.start()
        c_cp.start()
        wv_cp.start()
        wk_cp.start()
        moda_cp.start()
        x_cp(0).start()
        wq_cp.start()
        for i in range(1, n1):
            x_cp(i).start()
        wo_cp.start()
        modb_cp.start()
        wg_cp.start()
        wu_cp.start()
        wd_cp.start()

        wphi_cp.wait()
        wa = wphi_buf[...].reshape(Dh * Dh, H)
        sel = (_iota((H, D), 0) == _iota((H, D), 1) // Dh).astype(BF16)
        wb = _dot(wa, sel)
        wb = jnp.where(_iota((Dh * Dh, D), 0) // Dh == _iota((Dh * Dh, D), 1) % Dh, wb, 0.0)
        wb = wb.astype(BF16)
        rr = _iota((128, Dh * Dh), 0)
        rsel = ((rr % QW) // HQ == _iota((128, Dh * Dh), 1) % Dh).astype(BF16)
        rr = _iota((128, 128), 0)
        mask_k = (rr // QW) * HQ + rr % HQ == _iota((128, 128), 1) // Dh
        bd = []
        for g in range(G):
            t_k = _dot(rsel, wb[:, g * 128:(g + 1) * 128])
            bd.append(jnp.where(mask_k, t_k, 0.0).astype(BF16))

        def fold(cp_, off):
            cp_.wait()
            for g in range(G):
                w3t_buf[off + g * 128:off + (g + 1) * 128, :] = (LOG2E * _dot_nt(
                    bd[g], wqkv_buf[:, off + g * 128:off + (g + 1) * 128])).astype(BF16)

        wv_cp.wait()
        eye = (_iota((128, 128), 0) == _iota((128, 128), 1)).astype(BF16)
        for g in range(G):
            w3t_buf[2 * D + g * 128:2 * D + (g + 1) * 128, :] = _dot_nt(
                eye, wqkv_buf[:, 2 * D + g * 128:2 * D + (g + 1) * 128]).astype(BF16)
        fold(wk_cp, D)

        c_cp.wait()
        c32 = c_buf[...].astype(F32)
        sc8 = jnp.broadcast_to(c32 * jax.nn.sigmoid(c32), (8, D)).astype(BF16)
        moda_cp.wait()
        mod_buf[:, 0:2 * D] = _dot(sc8, wmod_buf[:, 0:2 * D])

        def ln1(i):
            sa = mod_buf[0:1, 0:D]
            ca = mod_buf[0:1, D:2 * D]
            r = pl.multiple_of(i * TM1, TM1)
            x = x_buf[pl.ds(r, TM1), :].astype(F32)
            h_buf[pl.ds(r, TM1), :] = (_layernorm(x) * (1.0 + ca) + sa).astype(BF16)

        def features(p):
            T = p.shape[1]
            blk = p.reshape(QW // 8, 8, T)

            def both(a, op):
                return op(a, pltpu.roll(a, HQ, axis=0))[None]

            mx = both(jnp.max(blk, axis=0), jnp.maximum)
            mn = both(jnp.min(blk, axis=0), jnp.minimum)
            ep = jnp.exp2(blk - mx)
            en = jnp.exp2(mn - blk)
            php = ep * (1.0 / both(jnp.sum(ep, axis=0), jnp.add))
            phn = en * (1.0 / both(jnp.sum(en, axis=0), jnp.add))
            return jnp.concatenate([php, phn], axis=0).reshape(2 * QW, T)

        def phase1(i, carry):
            @pl.when(i + 1 < n1)
            def _():
                x_cp(i + 1).wait()

            r = pl.multiple_of(i * TM1, TM1)
            h = h_buf[pl.ds(r, TM1), :]
            pqt = _dot_nt(w3t_buf[0:D, :], h)
            pkt = _dot_nt(w3t_buf[D:2 * D, :], h)
            for q in range(NQ):
                phq_buf[q, :, pl.ds(r, TM1)] = features(pqt[q * QW:(q + 1) * QW, :]).astype(BF16)
            vt = _dot_nt(w3t_buf[2 * D:3 * D, :], h).astype(BF16)
            ln1(jnp.minimum(i + 1, n1 - 1))
            for q in range(NQ):
                ph = features(pkt[q * QW:(q + 1) * QW, :])
                zs = ph[:, 0:128]
                for t in range(1, NL):
                    zs = zs + ph[:, t * 128:(t + 1) * 128]
                z_acc[q] += zs
                kv_acc[q] += _dot_nt(vt[q * QW:(q + 1) * QW, :], ph.astype(BF16))
            return carry

        x_cp(0).wait()
        ln1(0)
        fold(wq_cp, 0)
        kv_acc[...] = jnp.zeros(kv_acc.shape, F32)
        z_acc[...] = jnp.zeros(z_acc.shape, F32)
        jax.lax.fori_loop(0, n1, phase1, 0)

        wo_cp.wait()
        modb_cp.wait()
        wg_cp.wait()
        wu_cp.wait()
        wd_cp.wait()
        rr = _iota((128, 128), 0)
        cc = _iota((128, 128), 1)
        perm = ((rr // QW == cc // QW) & (rr % HQ == (cc % QW) // Dh)
                & ((rr % QW) // HQ == cc % Dh)).astype(BF16)
        mask_kv = _iota((QW, 2 * QW), 0) // Dh == _iota((QW, 2 * QW), 1) % HQ
        mask_z = ((_iota((16, 2 * QW), 0) % HQ == _iota((16, 2 * QW), 1) % HQ)
                  & (_iota((16, 2 * QW), 0) < 8))
        ones16 = jnp.ones((16, 128), BF16)
        for g in range(G):
            kvm = jnp.concatenate(
                [jnp.where(mask_kv, kv_acc[2 * g + t], 0.0).astype(BF16) for t in range(2)],
                axis=0)
            kvp = _dot(perm, kvm).astype(BF16)
            for t in range(2):
                q = 2 * g + t
                lhs_buf[q, 0:QW, :] = kvp[t * QW:(t + 1) * QW, :]
                zf = z_acc[q]
                zh = zf.astype(BF16)
                zl = (zf - zh.astype(F32)).astype(BF16)
                zr = _dot_nt(ones16, zh) + _dot_nt(ones16, zl)
                lhs_buf[q, QW:LR, :] = jnp.where(mask_z, zr, 0.0).astype(BF16)
            wop_buf[g * 128:(g + 1) * 128, :] = _dot(
                perm, wo_buf[g * 128:(g + 1) * 128, :]).astype(BF16)

        c32b = c_buf[...].astype(F32)
        sc8b = jnp.broadcast_to(c32b * jax.nn.sigmoid(c32b), (8, D)).astype(BF16)
        mod_buf[:, 2 * D:6 * D] = _dot(sc8b, wmod_buf[:, 2 * D:6 * D])

        def ln2_chunk(r, attn):
            ga = mod_buf[0:1, 2 * D:3 * D]
            sb = mod_buf[0:1, 3 * D:4 * D]
            cb = mod_buf[0:1, 4 * D:5 * D]
            x1 = x_buf[pl.ds(r, RC), :].astype(F32) + ga * attn
            x1_buf[pl.ds(r, RC), :] = x1
            h_buf[pl.ds(r, RC), :] = (_layernorm(x1) * (1.0 + cb) + sb).astype(BF16)

        def step(i_fin, i_ffn, i_front):
            jobs = []
            st = {"o": []}
            if i_front is not None:
                rf = pl.multiple_of(i_front * TM2, TM2)

                def job_a(q):
                    nd = _dot(lhs_buf[q], phq_buf[q, :, pl.ds(rf, TM2)])
                    num = nd[0:QW, :].reshape(QW // 8, 8, TM2)
                    rden = 1.0 / (nd[QW:QW + 8, :] + 1e-6)
                    st["o"].append((num * rden[None]).reshape(QW, TM2))

                def job_b():
                    ot = jnp.concatenate(st["o"], axis=0)
                    st["attn"] = _dot_tn(ot.astype(BF16), wop_buf[...])

                def job_c(c):
                    ln2_chunk(pl.multiple_of(rf + c * RC, RC),
                              st["attn"][c * RC:(c + 1) * RC, :])

                jobs = ([functools.partial(job_a, q) for q in range(NQ)] + [job_b]
                        + [functools.partial(job_c, c) for c in range(NC)])
            if i_fin is not None:
                r = pl.multiple_of(i_fin * TM2, TM2)
                gb = mod_buf[0:1, 5 * D:6 * D]
                out_buf[pl.ds(r, TM2), :] = (
                    x1_buf[pl.ds(r, TM2), :] + gb * acc_buf[pl.ds(r, TM2), :]).astype(BF16)
                out_cp(i_fin).start()
            if i_ffn is not None:
                r = pl.multiple_of(i_ffn * TM2, TM2)
                h2 = h_buf[pl.ds(r, TM2), :]
                acc = None
                k = 0
                for j in range(NF):
                    for _ in range(SCHED[j]):
                        if k < len(jobs):
                            jobs[k]()
                            k += 1
                    gt = _dot(h2, wg_buf[:, j * FC:(j + 1) * FC])
                    up = _dot(h2, wu_buf[:, j * FC:(j + 1) * FC])
                    act = (_gelu_tanh(gt) * up).astype(BF16)
                    d = _dot(act, wd_buf[j * FC:(j + 1) * FC, :])
                    acc = d if acc is None else acc + d
                while k < len(jobs):
                    jobs[k]()
                    k += 1
                acc_buf[pl.ds(r, TM2), :] = acc
            else:
                for jb in jobs:
                    jb()

        step(None, None, 0)
        step(None, 0, 1)

        def body(i, carry):
            step(i - 1, i, i + 1)
            return carry

        jax.lax.fori_loop(1, n2 - 1, body, 0, unroll=UNR2)
        step(n2 - 2, n2 - 1, None)
        step(n2 - 1, None, None)
        for i in range(n2):
            out_cp(i).wait()

    scratch = [
        pltpu.VMEM((S, D), BF16),
        pltpu.VMEM((D, 3 * D), BF16),
        pltpu.VMEM((Dh, Dh, H), BF16),
        pltpu.VMEM((D, D), BF16),
        pltpu.VMEM((D, F), BF16),
        pltpu.VMEM((D, F), BF16),
        pltpu.VMEM((F, D), BF16),
        pltpu.VMEM((1, D), BF16),
        pltpu.VMEM((D, 6 * D), BF16),
        pltpu.VMEM((3 * D, D), BF16),
        pltpu.VMEM((NQ, 2 * QW, S), BF16),
        pltpu.VMEM((NQ, QW, 2 * QW), F32),
        pltpu.VMEM((NQ, 2 * QW, 128), F32),
        pltpu.VMEM((NQ, LR, 2 * QW), BF16),
        pltpu.VMEM((D, D), BF16),
        pltpu.VMEM((8, 6 * D), F32),
        pltpu.VMEM((S, D), BF16),
        pltpu.VMEM((S, D), F32),
        pltpu.VMEM((S, D), F32),
        pltpu.VMEM((S, D), BF16),
        pltpu.SemaphoreType.DMA((NSEM,)),
    ]
    return kernel, scratch


@jax.jit
def pallas_adaLN_cond__linear_kernel_hedgehog__geglu_ffn__prompt_kernel(
    A_x: jax.Array,
    A_wqkv: jax.Array,
    A_w_phi: jax.Array,
    A_wo: jax.Array,
    B_x: jax.Array,
    B_w_gate: jax.Array,
    B_w_up: jax.Array,
    B_w_down: jax.Array,
    c: jax.Array,
    w_mod: jax.Array,
):
    B, S, D = A_x.shape
    H, Dh, _ = A_w_phi.shape
    F = B_w_gate.shape[1]
    TM1, TM2, FC, RC, UNR2 = 256, 256, 256, 64, 2
    SCHED = (0, 4, 4, 1, 2, 2, 0)
    assert B == 1 and Dh == 16 and H * Dh == D and D % 128 == 0
    assert S % TM1 == 0 and S % TM2 == 0 and S // TM2 >= 3 and F % FC == 0
    assert len(SCHED) == F // FC

    kernel, scratch = _make_kernel(S, D, H, Dh, F, TM1, TM2, FC, RC, SCHED, UNR2)
    any_spec = pl.BlockSpec(memory_space=pl.ANY)
    out = pl.pallas_call(
        kernel,
        out_shape=jax.ShapeDtypeStruct((S, D), BF16),
        in_specs=[any_spec] * 9,
        out_specs=any_spec,
        scratch_shapes=scratch,
        compiler_params=pltpu.CompilerParams(vmem_limit_bytes=100 * 1024 * 1024),
    )(
        A_x.reshape(S, D), A_wqkv, A_w_phi.transpose(1, 2, 0), A_wo,
        B_w_gate, B_w_up, B_w_down, c, w_mod,
    )
    return out.reshape(B, S, D)
```

```python
import functools

import jax
import jax.numpy as jnp
import jax.experimental.pallas as pl
import jax.experimental.pallas.tpu as pltpu

F32 = jnp.float32
BF16 = jnp.bfloat16

LOG2E = 1.4426950408889634

_NT = (((1,), (1,)), ((), ()))
_TN = (((0,), (0,)), ((), ()))


def _dot(a, b):
    return jnp.dot(a, b, preferred_element_type=F32)


def _dot_nt(a, b):
    return jax.lax.dot_general(a, b, _NT, preferred_element_type=F32)


def _dot_tn(a, b):
    return jax.lax.dot_general(a, b, _TN, preferred_element_type=F32)


def _iota(shape, dim):
    return jax.lax.broadcasted_iota(jnp.int32, shape, dim)


def _layernorm(x, eps=1e-5):
    m = jnp.mean(x, axis=-1, keepdims=True)
    xc = x - m
    v = jnp.mean(xc * xc, axis=-1, keepdims=True)
    return xc * jax.lax.rsqrt(v + eps)


def _gelu_tanh(x):
    c0 = 0.7978845608028654
    return 0.5 * x * (1.0 + jnp.tanh(c0 * (x + 0.044715 * (x * x * x))))


def _make_kernel(S, D, H, Dh, F, TM1, TM2, FC, RC, SCHED, UNR2):
    G = D // 128
    HQ = 4
    QW = HQ * Dh
    NQ = H // HQ
    n1 = S // TM1
    n2 = S // TM2
    NF = F // FC
    NL = TM1 // 128
    NC = TM2 // RC
    LR = QW + 16

    SEM_C, SEM_WPHI, SEM_WQ, SEM_WK, SEM_MODA, SEM_WV = 0, 1, 2, 3, 4, 5
    SEM_MODB, SEM_WO, SEM_WG, SEM_WU, SEM_WD = 6, 7, 8, 9, 10
    SEM_X = 11
    SEM_OUT = SEM_X + n1
    NSEM = SEM_OUT + n2

    def kernel(x_hbm, wqkv_hbm, wphi_hbm, wo_hbm, wg_hbm, wu_hbm, wd_hbm, c_hbm, wmod_hbm,
               out_hbm,
               x_buf, wqkv_buf, wphi_buf, wo_buf, wg_buf, wu_buf, wd_buf, c_buf, wmod_buf,
               w3t_buf, phq_buf, kv_acc, z_acc, lhs_buf, wop_buf, mod_buf,
               h_buf, x1_buf, acc_buf, out_buf, sems):

        def cp(src, dst, slot):
            return pltpu.make_async_copy(src, dst, sems.at[slot])

        c_cp = cp(c_hbm, c_buf, SEM_C)
        wphi_cp = cp(wphi_hbm, wphi_buf, SEM_WPHI)
        wq_cp = cp(wqkv_hbm.at[:, pl.ds(0, D)], wqkv_buf.at[:, pl.ds(0, D)], SEM_WQ)
        wk_cp = cp(wqkv_hbm.at[:, pl.ds(D, D)], wqkv_buf.at[:, pl.ds(D, D)], SEM_WK)
        wv_cp = cp(wqkv_hbm.at[:, pl.ds(2 * D, D)], wqkv_buf.at[:, pl.ds(2 * D, D)], SEM_WV)
        moda_cp = cp(wmod_hbm.at[:, pl.ds(0, 2 * D)], wmod_buf.at[:, pl.ds(0, 2 * D)], SEM_MODA)
        modb_cp = cp(wmod_hbm.at[:, pl.ds(2 * D, 4 * D)], wmod_buf.at[:, pl.ds(2 * D, 4 * D)],
                     SEM_MODB)
        wo_cp = cp(wo_hbm, wo_buf, SEM_WO)
        wg_cp = cp(wg_hbm, wg_buf, SEM_WG)
        wu_cp = cp(wu_hbm, wu_buf, SEM_WU)
        wd_cp = cp(wd_hbm, wd_buf, SEM_WD)

        def x_cp(i):
            r = pl.multiple_of(i * TM1, TM1)
            return cp(x_hbm.at[pl.ds(r, TM1), :], x_buf.at[pl.ds(r, TM1), :], SEM_X + i)

        def out_cp(i):
            r = pl.multiple_of(i * TM2, TM2)
            return cp(out_buf.at[pl.ds(r, TM2), :], out_hbm.at[pl.ds(r, TM2), :], SEM_OUT + i)

        wphi_cp.start()
        c_cp.start()
        wv_cp.start()
        wk_cp.start()
        moda_cp.start()
        x_cp(0).start()
        wq_cp.start()
        for i in range(1, n1):
            x_cp(i).start()
        wo_cp.start()
        modb_cp.start()
        wg_cp.start()
        wu_cp.start()
        wd_cp.start()

        wphi_cp.wait()
        wa = wphi_buf[...].reshape(Dh * Dh, H)
        sel = (_iota((H, D), 0) == _iota((H, D), 1) // Dh).astype(BF16)
        wb = _dot(wa, sel)
        wb = jnp.where(_iota((Dh * Dh, D), 0) // Dh == _iota((Dh * Dh, D), 1) % Dh, wb, 0.0)
        wb = wb.astype(BF16)
        rr = _iota((128, Dh * Dh), 0)
        rsel = ((rr % QW) // HQ == _iota((128, Dh * Dh), 1) % Dh).astype(BF16)
        rr = _iota((128, 128), 0)
        mask_k = (rr // QW) * HQ + rr % HQ == _iota((128, 128), 1) // Dh
        bd = []
        for g in range(G):
            t_k = _dot(rsel, wb[:, g * 128:(g + 1) * 128])
            bd.append(jnp.where(mask_k, t_k, 0.0).astype(BF16))

        def fold(cp_, off):
            cp_.wait()
            for g in range(G):
                w3t_buf[off + g * 128:off + (g + 1) * 128, :] = (LOG2E * _dot_nt(
                    bd[g], wqkv_buf[:, off + g * 128:off + (g + 1) * 128])).astype(BF16)

        rr = _iota((128, 128), 0)
        cc = _iota((128, 128), 1)
        perm = ((rr // QW == cc // QW) & (rr % HQ == (cc % QW) // Dh)
                & ((rr % QW) // HQ == cc % Dh)).astype(BF16)
        wv_cp.wait()
        for g in range(G):
            w3t_buf[2 * D + g * 128:2 * D + (g + 1) * 128, :] = _dot_nt(
                perm, wqkv_buf[:, 2 * D + g * 128:2 * D + (g + 1) * 128]).astype(BF16)
        fold(wk_cp, D)

        c_cp.wait()
        c32 = c_buf[...].astype(F32)
        sc8 = jnp.broadcast_to(c32 * jax.nn.sigmoid(c32), (8, D)).astype(BF16)
        moda_cp.wait()
        mod_buf[:, 0:2 * D] = _dot(sc8, wmod_buf[:, 0:2 * D])

        def ln1(i):
            sa = mod_buf[0:1, 0:D]
            ca = mod_buf[0:1, D:2 * D]
            r = pl.multiple_of(i * TM1, TM1)
            x = x_buf[pl.ds(r, TM1), :].astype(F32)
            h_buf[pl.ds(r, TM1), :] = (_layernorm(x) * (1.0 + ca) + sa).astype(BF16)

        def features(p):
            T = p.shape[1]
            blk = p.reshape(QW // 8, 8, T)

            def both(a, op):
                return op(a, pltpu.roll(a, HQ, axis=0))[None]

            mx = both(jnp.max(blk, axis=0), jnp.maximum)
            mn = both(jnp.min(blk, axis=0), jnp.minimum)
            ep = jnp.exp2(blk - mx)
            en = jnp.exp2(mn - blk)
            php = ep * (1.0 / both(jnp.sum(ep, axis=0), jnp.add))
            phn = en * (1.0 / both(jnp.sum(en, axis=0), jnp.add))
            return jnp.concatenate([php, phn], axis=0).reshape(2 * QW, T)

        def phase1(i, carry):
            @pl.when(i + 1 < n1)
            def _():
                x_cp(i + 1).wait()

            r = pl.multiple_of(i * TM1, TM1)
            h = h_buf[pl.ds(r, TM1), :]
            pqt = _dot_nt(w3t_buf[0:D, :], h)
            pkt = _dot_nt(w3t_buf[D:2 * D, :], h)
            for q in range(NQ):
                phq_buf[q, :, pl.ds(r, TM1)] = features(pqt[q * QW:(q + 1) * QW, :]).astype(BF16)
            vt = _dot_nt(w3t_buf[2 * D:3 * D, :], h).astype(BF16)
            ln1(jnp.minimum(i + 1, n1 - 1))
            for q in range(NQ):
                ph = features(pkt[q * QW:(q + 1) * QW, :])
                zs = ph[:, 0:128]
                for t in range(1, NL):
                    zs = zs + ph[:, t * 128:(t + 1) * 128]
                z_acc[q] += zs
                kv_acc[q] += _dot_nt(vt[q * QW:(q + 1) * QW, :], ph.astype(BF16))
            return carry

        x_cp(0).wait()
        ln1(0)
        fold(wq_cp, 0)
        kv_acc[...] = jnp.zeros(kv_acc.shape, F32)
        z_acc[...] = jnp.zeros(z_acc.shape, F32)
        jax.lax.fori_loop(0, n1, phase1, 0)

        wo_cp.wait()
        modb_cp.wait()
        wg_cp.wait()
        wu_cp.wait()
        wd_cp.wait()
        mask_kv = _iota((QW, 2 * QW), 0) % HQ == _iota((QW, 2 * QW), 1) % HQ
        mask_z = ((_iota((16, 2 * QW), 0) % HQ == _iota((16, 2 * QW), 1) % HQ)
                  & (_iota((16, 2 * QW), 0) < 8))
        ones16 = jnp.ones((16, 128), BF16)
        for q in range(NQ):
            lhs_buf[q, 0:QW, :] = jnp.where(mask_kv, kv_acc[q], 0.0).astype(BF16)
            zf = z_acc[q]
            zh = zf.astype(BF16)
            zl = (zf - zh.astype(F32)).astype(BF16)
            zr = _dot_nt(ones16, zh) + _dot_nt(ones16, zl)
            lhs_buf[q, QW:LR, :] = jnp.where(mask_z, zr, 0.0).astype(BF16)
        rr = _iota((128, 128), 0)
        cc = _iota((128, 128), 1)
        perm = ((rr // QW == cc // QW) & (rr % HQ == (cc % QW) // Dh)
                & ((rr % QW) // HQ == cc % Dh)).astype(BF16)
        for g in range(G):
            wop_buf[g * 128:(g + 1) * 128, :] = _dot(
                perm, wo_buf[g * 128:(g + 1) * 128, :]).astype(BF16)

        c32b = c_buf[...].astype(F32)
        sc8b = jnp.broadcast_to(c32b * jax.nn.sigmoid(c32b), (8, D)).astype(BF16)
        mod_buf[:, 2 * D:6 * D] = _dot(sc8b, wmod_buf[:, 2 * D:6 * D])

        def ln2_chunk(r, attn):
            ga = mod_buf[0:1, 2 * D:3 * D]
            sb = mod_buf[0:1, 3 * D:4 * D]
            cb = mod_buf[0:1, 4 * D:5 * D]
            x1 = x_buf[pl.ds(r, RC), :].astype(F32) + ga * attn
            x1_buf[pl.ds(r, RC), :] = x1
            h_buf[pl.ds(r, RC), :] = (_layernorm(x1) * (1.0 + cb) + sb).astype(BF16)

        def step(i_fin, i_ffn, i_front):
            jobs = []
            st = {"o": []}
            if i_front is not None:
                rf = pl.multiple_of(i_front * TM2, TM2)

                def job_a(q):
                    nd = _dot(lhs_buf[q], phq_buf[q, :, pl.ds(rf, TM2)])
                    num = nd[0:QW, :].reshape(QW // 8, 8, TM2)
                    rden = 1.0 / (nd[QW:QW + 8, :] + 1e-6)
                    st["o"].append((num * rden[None]).reshape(QW, TM2))

                def job_b():
                    ot = jnp.concatenate(st["o"], axis=0)
                    st["attn"] = _dot_tn(ot.astype(BF16), wop_buf[...])

                def job_c(c):
                    ln2_chunk(pl.multiple_of(rf + c * RC, RC),
                              st["attn"][c * RC:(c + 1) * RC, :])

                jobs = ([functools.partial(job_a, q) for q in range(NQ)] + [job_b]
                        + [functools.partial(job_c, c) for c in range(NC)])
            if i_fin is not None:
                r = pl.multiple_of(i_fin * TM2, TM2)
                gb = mod_buf[0:1, 5 * D:6 * D]
                out_buf[pl.ds(r, TM2), :] = (
                    x1_buf[pl.ds(r, TM2), :] + gb * acc_buf[pl.ds(r, TM2), :]).astype(BF16)
                out_cp(i_fin).start()
            if i_ffn is not None:
                r = pl.multiple_of(i_ffn * TM2, TM2)
                h2 = h_buf[pl.ds(r, TM2), :]
                acc = None
                k = 0
                for j in range(NF):
                    for _ in range(SCHED[j]):
                        if k < len(jobs):
                            jobs[k]()
                            k += 1
                    gt = _dot(h2, wg_buf[:, j * FC:(j + 1) * FC])
                    up = _dot(h2, wu_buf[:, j * FC:(j + 1) * FC])
                    act = (_gelu_tanh(gt) * up).astype(BF16)
                    d = _dot(act, wd_buf[j * FC:(j + 1) * FC, :])
                    acc = d if acc is None else acc + d
                while k < len(jobs):
                    jobs[k]()
                    k += 1
                acc_buf[pl.ds(r, TM2), :] = acc
            else:
                for jb in jobs:
                    jb()

        step(None, None, 0)
        step(None, 0, 1)

        def body(i, carry):
            step(i - 1, i, i + 1)
            return carry

        jax.lax.fori_loop(1, n2 - 1, body, 0, unroll=UNR2)
        step(n2 - 2, n2 - 1, None)
        step(n2 - 1, None, None)
        for i in range(n2):
            out_cp(i).wait()

    scratch = [
        pltpu.VMEM((S, D), BF16),
        pltpu.VMEM((D, 3 * D), BF16),
        pltpu.VMEM((Dh, Dh, H), BF16),
        pltpu.VMEM((D, D), BF16),
        pltpu.VMEM((D, F), BF16),
        pltpu.VMEM((D, F), BF16),
        pltpu.VMEM((F, D), BF16),
        pltpu.VMEM((1, D), BF16),
        pltpu.VMEM((D, 6 * D), BF16),
        pltpu.VMEM((3 * D, D), BF16),
        pltpu.VMEM((NQ, 2 * QW, S), BF16),
        pltpu.VMEM((NQ, QW, 2 * QW), F32),
        pltpu.VMEM((NQ, 2 * QW, 128), F32),
        pltpu.VMEM((NQ, LR, 2 * QW), BF16),
        pltpu.VMEM((D, D), BF16),
        pltpu.VMEM((8, 6 * D), F32),
        pltpu.VMEM((S, D), BF16),
        pltpu.VMEM((S, D), F32),
        pltpu.VMEM((S, D), F32),
        pltpu.VMEM((S, D), BF16),
        pltpu.SemaphoreType.DMA((NSEM,)),
    ]
    return kernel, scratch


@jax.jit
def pallas_adaLN_cond__linear_kernel_hedgehog__geglu_ffn__prompt_kernel(
    A_x: jax.Array,
    A_wqkv: jax.Array,
    A_w_phi: jax.Array,
    A_wo: jax.Array,
    B_x: jax.Array,
    B_w_gate: jax.Array,
    B_w_up: jax.Array,
    B_w_down: jax.Array,
    c: jax.Array,
    w_mod: jax.Array,
):
    B, S, D = A_x.shape
    H, Dh, _ = A_w_phi.shape
    F = B_w_gate.shape[1]
    TM1, TM2, FC, RC, UNR2 = 256, 256, 256, 64, 2
    SCHED = (0, 4, 4, 1, 2, 2, 0)
    assert B == 1 and Dh == 16 and H * Dh == D and D % 128 == 0
    assert S % TM1 == 0 and S % TM2 == 0 and S // TM2 >= 3 and F % FC == 0
    assert len(SCHED) == F // FC

    kernel, scratch = _make_kernel(S, D, H, Dh, F, TM1, TM2, FC, RC, SCHED, UNR2)
    any_spec = pl.BlockSpec(memory_space=pl.ANY)
    out = pl.pallas_call(
        kernel,
        out_shape=jax.ShapeDtypeStruct((S, D), BF16),
        in_specs=[any_spec] * 9,
        out_specs=any_spec,
        scratch_shapes=scratch,
        compiler_params=pltpu.CompilerParams(vmem_limit_bytes=100 * 1024 * 1024),
    )(
        A_x.reshape(S, D), A_wqkv, A_w_phi.transpose(1, 2, 0), A_wo,
        B_w_gate, B_w_up, B_w_down, c, w_mod,
    )
    return out.reshape(B, S, D)
```
